```python
import jax
import jax.numpy as jnp

def _softmax(x, axis=-1):
    return jax.nn.softmax(x, axis=axis)

def _gelu(x):
    return jax.nn.gelu(x, approximate=True)

def _silu(x):
    return jax.nn.silu(x)

def _sigmoid(x):
    return jax.nn.sigmoid(x)

def _layernorm(x, axis=-1, eps=1e-05):
    m = jnp.mean(x, axis=axis, keepdims=True)
    v = jnp.var(x, axis=axis, keepdims=True)
    return (x - m) / jnp.sqrt(v + eps)

def _scatter_add(tgt, idx, src, axis=0):
    return tgt.at[idx].add(src)

def _segment_sum(src, seg, n):
    return jax.ops.segment_sum(src, seg, n)

class _Rng:

    def __init__(self, key):
        self._k = key

    def _next(self):
        self._k, sub = jax.random.split(self._k)
        return sub

    def normal(self, shape):
        return jax.random.normal(self._next(), shape, dtype=jnp.bfloat16)

    def randint(self, lo, hi, shape):
        return jax.random.randint(self._next(), shape, lo, hi, dtype=jnp.int32)

    def uniform(self, shape, lo=0.0, hi=1.0):
        return jax.random.uniform(self._next(), shape, jnp.bfloat16, lo, hi)

    def permutation(self, n):
        return jax.random.permutation(self._next(), n)
kernel_name = 'interleave_layers__sliding_local_dilated__mixer_gmlp__prompt'

def setup_inputs():
    _rng = _Rng(jax.random.key(int.from_bytes(__import__("os").urandom(4), "little")))
    _w = lambda a: (lambda t: t.astype(jnp.bfloat16) if jnp.issubdtype(t.dtype, jnp.floating) else t)(jnp.asarray(a))

    def _A_setup():
        B, S, D = (1, 2048, 576)
        return {'x': _w((lambda *s: _rng.normal(s) * 0.05)(B, S, D)), 'wqkv': _w((lambda *s: _rng.normal(s) * 0.05)(D, 3 * D)), 'wo': _w((lambda *s: _rng.normal(s) * 0.05)(D, D))}
    _A_in = _A_setup()

    def _B_setup():
        B, S, D, F = (1, 2048, 576, 4608)
        Fh = F // 2
        return {'x': _w((lambda *s: _rng.normal(s) * 0.05)(B, S, D)), 'w_in': _w((lambda *s: _rng.normal(s) * 0.05)(D, 2 * Fh)), 'w_sp': _w(0.01 * (lambda *s: _rng.normal(s) * 0.05)(S, S)), 'b_sp': _w(1.0 + 0.01 * (lambda *s: _rng.normal(s) * 0.05)(S)), 'w_out': _w((lambda *s: _rng.normal(s) * 0.05)(Fh, D))}
    _B_in = _B_setup()
    return {'A_x': _A_in['x'], 'A_wqkv': _A_in['wqkv'], 'A_wo': _A_in['wo'], 'B_x': _B_in['x'], 'B_w_in': _B_in['w_in'], 'B_w_sp': _B_in['w_sp'], 'B_b_sp': _B_in['b_sp'], 'B_w_out': _B_in['w_out']}

def reference(A_x, A_wqkv, A_wo, B_x, B_w_in, B_w_sp, B_b_sp, B_w_out):

    def _A_ref(x, wqkv, wo):
        B, S, D = x.shape
        H = 32
        Dh = D // H
        W, dil = (8, 2)
        qkv = (lambda x, *d: x.transpose(*d))((x @ wqkv).reshape(B, S, 3, H, Dh), 2, 0, 3, 1, 4)
        q, k, v = (qkv[0], qkv[1], qkv[2])
        scale = Dh ** (-0.5)
        pos = jnp.arange(S)
        off = jnp.arange(W) * dil
        idx = pos[:, None] - off[None, :]
        mask = idx >= 0
        idx_c = jnp.where(mask, idx, 0).reshape(-1)
        kg = k[:, :, idx_c, :].reshape(B, H, S, W, Dh)
        vg = v[:, :, idx_c, :].reshape(B, H, S, W, Dh)
        logits = jnp.einsum('bhsd,bhswd->bhsw', q, kg) * scale
        logits = jnp.where(mask[None, None, :, :], logits, -1000000000.0)
        attn = _softmax(logits, axis=-1)
        o = jnp.einsum('bhsw,bhswd->bhsd', attn, vg)
        return (lambda x, *d: x.transpose(*d))(o, 0, 2, 1, 3).reshape(B, S, D) @ wo

    def _B_ref(x, w_in, w_sp, b_sp, w_out):
        B, S, D = x.shape
        F = w_in.shape[-1]
        Fh = F // 2
        z = _gelu(jnp.einsum('bsd,df->bsf', x, w_in))
        z1 = z[..., :Fh].copy()
        z2 = _layernorm(z[..., Fh:], axis=-1)
        g = jnp.einsum('ts,bsf->btf', w_sp, z2) + b_sp[None, :, None]
        return jnp.einsum('bsf,fd->bsd', z1 * g, w_out)
    x = A_x
    x = x + _A_ref(_layernorm(x, axis=-1), A_wqkv, A_wo)
    x = x + _B_ref(_layernorm(x, axis=-1), B_w_in, B_w_sp, B_b_sp, B_w_out)
    x = x + _A_ref(_layernorm(x, axis=-1), A_wqkv, A_wo)
    x = x + _B_ref(_layernorm(x, axis=-1), B_w_in, B_w_sp, B_b_sp, B_w_out)
    return x
```

```python
import numpy as np
import jax
import jax.numpy as jnp
from jax import lax
import jax.experimental.pallas as pl
import jax.experimental.pallas.tpu as pltpu

S = 2048
D = 576
H = 32
DH = 18
W = 8
DIL = 2
FH = 2304
DP = 640
NC = DP // 128
HALO = 16
EPS = 1e-5
TM = 256
TB = 256
RS = 32
ZC = 768
_END = object()
BF = jnp.bfloat16
F32 = jnp.float32
GC = float(np.sqrt(2.0 / np.pi))


def _dot(a, b):
    return jnp.dot(a, b, preferred_element_type=F32)


def _dot_nt(a, b):
    return lax.dot_general(a, b, (((1,), (1,)), ((), ())), preferred_element_type=F32)


def _ln0(x):
    m = jnp.mean(x, axis=0, keepdims=True)
    xc = x - m
    v = jnp.mean(xc * xc, axis=0, keepdims=True)
    return xc * lax.rsqrt(v + EPS)


def _gelu2(x):
    t = jnp.tanh(x * (GC + (GC * 0.044715) * (x * x)))
    return x * t + x


def _kernel(x_hbm, wqkv_hbm, wo_hbm, win_hbm, wsp_hbm, b_ref, wout_hbm, out_hbm,
            xio, xr, xn, wqkv_raw, wqkv_p, wo_raw, wo_p, win, wsp, wout,
            q_s, k_s, v_s, o_s, z2, bb, sems, osems):
    cps = [pltpu.make_async_copy(src, dst, sems.at[i]) for i, (src, dst) in enumerate([
        (wqkv_hbm, wqkv_raw), (x_hbm.at[0], xio), (wo_hbm, wo_raw),
        (win_hbm, win), (wsp_hbm, wsp), (wout_hbm, wout)])]
    for c in cps:
        c.start()

    k_s[:, 0:HALO, :] = jnp.zeros((NC, HALO, 128), F32)
    v_s[:, 0:HALO, :] = jnp.zeros((NC, HALO, 128), F32)
    bb[...] = jnp.broadcast_to(b_ref[...].astype(F32) * 0.5, (128, S)).T

    cps[0].wait()

    def perm_rows(tmp, c0):
        cols = []
        for c in range(NC):
            parts = [tmp[c, pl.ds(c0 + g * 8 * DH + d, 8, stride=DH), :]
                     for d in range(DH) for g in range(H // 8)]
            parts.append(jnp.zeros((DP - D, 128), F32))
            cols.append(jnp.concatenate(parts, axis=0))
        return cols

    tmp = q_s
    for c in range(NC):
        r = min(128, D - c * 128)
        blk = wqkv_raw[c * 128:c * 128 + r, :].astype(F32)
        if r < 128:
            blk = jnp.concatenate([blk, jnp.zeros((128 - r, 3 * D), F32)], axis=0)
        tmp[c, 0:3 * D, :] = blk.T
    for sec in range(3):
        cols = perm_rows(tmp, sec * D)
        for c in range(NC):
            r = min(128, D - c * 128)
            wqkv_p[c * 128:c * 128 + r, sec * DP:(sec + 1) * DP] = cols[c].T[0:r].astype(BF)

    cps[2].wait()
    wo_f = wo_raw[...].astype(F32)
    for c in range(NC):
        r = min(128, D - c * 128)
        tmp[c, 0:D, 0:r] = wo_f[:, c * 128:c * 128 + r]
    cols = perm_rows(tmp, 0)
    wo_p[...] = jnp.concatenate([t.T for t in cols], axis=0)[0:D].astype(BF)

    cps[1].wait()
    xr[...] = xio[...].astype(F32)

    scale = DH ** -0.5
    NB = S // TM

    def qkv_block(i):
        cs = pl.ds(i * TM, TM)
        h = _ln0(xr[:, cs]).T.astype(BF)
        yield
        for sec, (dst, off) in enumerate([(q_s, 0), (k_s, HALO), (v_s, HALO)]):
            t = _dot(h, wqkv_p[:, sec * DP:(sec + 1) * DP])
            if sec == 0:
                t = t * scale
            for c in range(NC):
                dst[c, pl.ds(i * TM + off, TM), :] = t[:, c * 128:(c + 1) * 128]
            yield

    def attn_block(i):
        for sb in range(TM // RS):
            r = i * TM + sb * RS
            qs = [q_s[c, pl.ds(r, RS), :] for c in range(NC)]
            ls = []
            for w in range(W):
                p = None
                for c in range(NC):
                    t = qs[c] * k_s[c, pl.ds(r + HALO - DIL * w, RS), :]
                    p = t if p is None else p + t
                p = p + pltpu.roll(p, 64, 1)
                p = p + pltpu.roll(p, 32, 1)
                if r < DIL * w:
                    pos = r + lax.broadcasted_iota(jnp.int32, (RS, 128), 0)
                    p = jnp.where(pos >= DIL * w, p, -1e9)
                ls.append(p)
            m = ls[0]
            for w in range(1, W):
                m = jnp.maximum(m, ls[w])
            es = [jnp.exp(l - m) for l in ls]
            den = es[0]
            for w in range(1, W):
                den = den + es[w]
            inv = 1.0 / den
            for c in range(NC):
                o = None
                for w in range(W):
                    t = es[w] * v_s[c, pl.ds(r + HALO - DIL * w, RS), :]
                    o = t if o is None else o + t
                o_s[pl.ds(r, RS), c * 128:(c + 1) * 128] = (o * inv).astype(BF)
            yield

    def post_block(i):
        cs = pl.ds(i * TM, TM)
        x = xr[:, cs] + _dot_nt(wo_p[...], o_s[cs, :])
        xr[:, cs] = x
        h = _ln0(x).T.astype(BF)
        xn[cs, :] = h
        yield
        zs = []
        for j in range(FH // ZC):
            zs.append(_gelu2(_dot(h, win[:, FH + j * ZC:FH + (j + 1) * ZC])))
            yield
        z = jnp.concatenate(zs, axis=1)
        m = jnp.mean(z, axis=-1, keepdims=True)
        zc = z - m
        v = jnp.mean(zc * zc, axis=-1, keepdims=True)
        z2[cs, :] = (zc * (0.5 * lax.rsqrt(v + 4.0 * EPS))).astype(BF)
        yield

    def interleave(gens):
        while gens:
            gens = [g for g in gens if next(g, _END) is not _END]

    def layer(li, carry):
        for i in range(-1, NB + 1):
            if i == 1:
                @pl.when(li == 0)
                def _():
                    cps[3].wait()
            gens = []
            if i + 1 < NB:
                gens.append(qkv_block(i + 1))
            if 0 <= i - 1:
                gens.append(post_block(i - 1))
            if 0 <= i < NB:
                gens.append(attn_block(i))
            interleave(gens)

        @pl.when(li == 0)
        def _():
            cps[4].wait()
            cps[5].wait()

        def b2(i, _):
            rows = pl.ds(pl.multiple_of(i * TB, TB), TB)
            z1 = _gelu2(_dot(xn[rows, :], win[:, :FH]))
            g = _dot(wsp[rows, :], z2[...])
            b = bb[rows, :]
            g = g + jnp.concatenate([b] * (FH // 128), axis=1)
            x = xr[:, rows] + _dot_nt(wout[...], (z1 * g).astype(BF))
            xr[:, rows] = x

            @pl.when(li == 1)
            def _():
                xio[:, rows] = xr[:, rows].astype(BF)
                pltpu.make_async_copy(xio.at[:, rows], out_hbm.at[0, :, rows], osems.at[i]).start()
            return 0
        lax.fori_loop(0, S // TB, b2, 0)
        return 0

    lax.fori_loop(0, 2, layer, 0)
    for i in range(S // TB):
        rows = pl.ds(i * TB, TB)
        pltpu.make_async_copy(xio.at[:, rows], out_hbm.at[0, :, rows], osems.at[i]).wait()


@jax.jit
def pallas_interleave_layers__sliding_local_dilated__mixer_gmlp__prompt_kernel(
    A_x: jax.Array,
    A_wqkv: jax.Array,
    A_wo: jax.Array,
    B_x: jax.Array,
    B_w_in: jax.Array,
    B_w_sp: jax.Array,
    B_b_sp: jax.Array,
    B_w_out: jax.Array,
):
    hbm = pl.BlockSpec(memory_space=pltpu.HBM)
    V = pltpu.VMEM
    out_t = pl.pallas_call(
        _kernel,
        out_shape=jax.ShapeDtypeStruct((1, D, S), BF),
        in_specs=[hbm, hbm, hbm, hbm, hbm, pl.BlockSpec(memory_space=pltpu.VMEM), hbm],
        out_specs=hbm,
        scratch_shapes=[
            V((D, S), BF), V((D, S), F32), V((S, D), BF),
            V((D, 3 * D), BF), V((D, 3 * DP), BF), V((D, D), BF), V((D, DP), BF),
            V((D, 2 * FH), BF), V((S, S), BF), V((D, FH), BF),
            V((NC, S, 128), F32), V((NC, S + HALO, 128), F32), V((NC, S + HALO, 128), F32),
            V((S, DP), BF), V((S, FH), BF), V((S, 128), F32),
            pltpu.SemaphoreType.DMA((6,)), pltpu.SemaphoreType.DMA((S // TB,)),
        ],
        compiler_params=pltpu.CompilerParams(vmem_limit_bytes=110 * 1024 * 1024),
    )(jnp.swapaxes(A_x, 1, 2), A_wqkv, A_wo, B_w_in, B_w_sp, B_b_sp.reshape(1, S), B_w_out.T)
    return jnp.swapaxes(out_t, 1, 2)
```
